```python
import os as _os
_os.environ.setdefault("JAX_PLATFORMS", "cpu")
import jax
import jax.numpy as jnp

def _softmax(x, axis=-1):
    return jax.nn.softmax(x, axis=axis)
def _gelu(x):
    return jax.nn.gelu(x, approximate=True)
def _silu(x):
    return jax.nn.silu(x)
def _sigmoid(x):
    return jax.nn.sigmoid(x)
def _layernorm(x, axis=-1, eps=1e-5):
    m = jnp.mean(x, axis=axis, keepdims=True)
    v = jnp.var(x, axis=axis, keepdims=True)
    return (x - m) / jnp.sqrt(v + eps)
def _scatter_add(tgt, idx, src, axis=0):
    return tgt.at[idx].add(src)
def _segment_sum(src, seg, n):
    return jax.ops.segment_sum(src, seg, n)
class _Rng:
    def __init__(self, key):
        self._k = key
    def _next(self):
        self._k, sub = jax.random.split(self._k)
        return sub
    def normal(self, shape):
        return jax.random.normal(self._next(), shape, dtype=jnp.bfloat16)
    def randint(self, lo, hi, shape):
        return jax.random.randint(self._next(), shape, lo, hi, dtype=jnp.int32)
    def uniform(self, shape, lo=0.0, hi=1.0):
        return jax.random.uniform(self._next(), shape, jnp.bfloat16, lo, hi)
    def permutation(self, n):
        return jax.random.permutation(self._next(), n)


kernel_name = 'concat_heads__gqa_block_cached__gqa_block_cached__near_ridge'

def setup_inputs():
    _rng = _Rng(jax.random.key(int.from_bytes(__import__("os").urandom(4), "little")))
    _w = (lambda a: (lambda t: t.astype(jnp.bfloat16) if jnp.issubdtype(t.dtype, jnp.floating) else t)(jnp.asarray(a)))
    def _A_setup():
        B, Sq, D = 8, 240, 640
        Hq, Hkv, Sk, Dh = 32, 32, 1024, 192
        assert Hq % Hkv == 0, (Hq, Hkv)
        return {
            "x": _w((lambda *s: _rng.normal(s) * 0.8)(B, Sq, D)),
            "k_cache": _w((lambda *s: _rng.normal(s) * 0.8)(B, Hkv, Sk, Dh)),
            "v_cache": _w((lambda *s: _rng.normal(s) * 0.05)(B, Hkv, Sk, Dh)),
            "wq": _w((lambda *s: _rng.normal(s) * 0.8)(D, Hq * Dh) * (D ** -0.5)),
            "wo": _w((lambda *s: _rng.normal(s) * 0.05)(Hq * Dh, D) * ((Hq * Dh) ** -0.5)),
        }
    _A_in = _A_setup()

    def _B_setup():
        B, Sq, D = 8, 240, 640
        Hq, Hkv, Sk, Dh = 32, 32, 1024, 192
        assert Hq % Hkv == 0, (Hq, Hkv)
        return {
            "x": _w((lambda *s: _rng.normal(s) * 0.8)(B, Sq, D)),
            "k_cache": _w((lambda *s: _rng.normal(s) * 0.8)(B, Hkv, Sk, Dh)),
            "v_cache": _w((lambda *s: _rng.normal(s) * 0.05)(B, Hkv, Sk, Dh)),
            "wq": _w((lambda *s: _rng.normal(s) * 0.8)(D, Hq * Dh) * (D ** -0.5)),
            "wo": _w((lambda *s: _rng.normal(s) * 0.05)(Hq * Dh, D) * ((Hq * Dh) ** -0.5)),
        }
    _B_in = _B_setup()

    return {
        "A_x": _A_in["x"],
        "A_k_cache": _A_in["k_cache"],
        "A_v_cache": _A_in["v_cache"],
        "A_wq": _A_in["wq"],
        "A_wo": _A_in["wo"],
        "B_x": _B_in["x"],
        "B_k_cache": _B_in["k_cache"],
        "B_v_cache": _B_in["v_cache"],
        "B_wq": _B_in["wq"],
        "B_wo": _B_in["wo"],
    }

def reference(A_x, A_k_cache, A_v_cache, A_wq, A_wo, B_x, B_k_cache, B_v_cache, B_wq, B_wo):
    def _A_ref(x, k_cache, v_cache, wq, wo):
        B, Sq, D = x.shape
        Hq, Dh = 32, 192
        Hkv = k_cache.shape[1]
        rep = Hq // Hkv
        q = (lambda x, *d: x.transpose(*d))((x @ wq).reshape(B, Sq, Hq, Dh), 0, 2, 1, 3)
        k = jnp.repeat(k_cache, rep, axis=1)
        v = jnp.repeat(v_cache, rep, axis=1)
        scores = jnp.einsum("bhqd,bhkd->bhqk", q, k) * (Dh ** -0.5)
        p = _softmax(scores, axis=-1)
        o = jnp.einsum("bhqk,bhkd->bhqd", p, v)
        return (lambda x, *d: x.transpose(*d))(o, 0, 2, 1, 3).reshape(B, Sq, Hq * Dh) @ wo

    def _B_ref(x, k_cache, v_cache, wq, wo):
        B, Sq, D = x.shape
        Hq, Dh = 32, 192
        Hkv = k_cache.shape[1]
        rep = Hq // Hkv
        q = (lambda x, *d: x.transpose(*d))((x @ wq).reshape(B, Sq, Hq, Dh), 0, 2, 1, 3)
        k = jnp.repeat(k_cache, rep, axis=1)
        v = jnp.repeat(v_cache, rep, axis=1)
        scores = jnp.einsum("bhqd,bhkd->bhqk", q, k) * (Dh ** -0.5)
        p = _softmax(scores, axis=-1)
        o = jnp.einsum("bhqk,bhkd->bhqd", p, v)
        return (lambda x, *d: x.transpose(*d))(o, 0, 2, 1, 3).reshape(B, Sq, Hq * Dh) @ wo

    a = _A_ref(A_x, A_k_cache, A_v_cache, A_wq, A_wo)
    b = _B_ref(B_x, B_k_cache, B_v_cache, B_wq, B_wo)
    return jnp.concatenate([a, b], axis=-1)
```

```python
import functools

import jax
import jax.numpy as jnp
import jax.experimental.pallas as pl
import jax.experimental.pallas.tpu as pltpu

HPS = 2


def _kernel(ax_ref, ak_ref, av_ref, awq_ref, awo_ref,
            bx_ref, bk_ref, bv_ref, bwq_ref, bwo_ref,
            o_ref, acc_ref, *, dh, d_model, scale):
    hp = pl.program_id(0)
    b = pl.program_id(1)
    nhp = pl.num_programs(0)

    for prob, (x_ref, k_ref, v_ref, wq_ref, wo_ref) in enumerate((
            (ax_ref, ak_ref, av_ref, awq_ref, awo_ref),
            (bx_ref, bk_ref, bv_ref, bwq_ref, bwo_ref))):
        x = x_ref[b]
        q = jnp.dot(x, wq_ref[...], preferred_element_type=jnp.float32)
        q = (q * scale).astype(jnp.bfloat16)
        outs = []
        for j in range(HPS):
            qj = q[:, j * dh:(j + 1) * dh]
            s = jax.lax.dot_general(qj, k_ref[0, j], (((1,), (1,)), ((), ())),
                                    preferred_element_type=jnp.float32)
            m = jnp.max(s, axis=-1, keepdims=True)
            p = jnp.exp(s - m)
            l = jnp.sum(p, axis=-1, keepdims=True)
            oj = jnp.dot(p.astype(jnp.bfloat16), v_ref[0, j],
                         preferred_element_type=jnp.float32)
            outs.append((oj / l).astype(jnp.bfloat16))
        o = jnp.concatenate(outs, axis=-1)
        contrib = jnp.dot(o, wo_ref[...], preferred_element_type=jnp.float32)
        cols = slice(prob * d_model, (prob + 1) * d_model)

        @pl.when(hp == 0)
        def _():
            acc_ref[b, :, cols] = contrib

        @pl.when(hp > 0)
        def _():
            acc_ref[b, :, cols] += contrib

    @pl.when(hp == nhp - 1)
    def _():
        o_ref[b] = acc_ref[b].astype(o_ref.dtype)


@jax.jit
def pallas_concat_heads__gqa_block_cached__gqa_block_cached__near_ridge_kernel(
    A_x: jax.Array,
    A_k_cache: jax.Array,
    A_v_cache: jax.Array,
    A_wq: jax.Array,
    A_wo: jax.Array,
    B_x: jax.Array,
    B_k_cache: jax.Array,
    B_v_cache: jax.Array,
    B_wq: jax.Array,
    B_wo: jax.Array,
):
    nb, sq, d_model = A_x.shape
    _, hkv, sk, dh = A_k_cache.shape
    hq = A_wq.shape[1] // dh
    assert hq == hkv and hq % HPS == 0
    nhp = hq // HPS
    w = HPS * dh

    x_spec = pl.BlockSpec((nb, sq, d_model), lambda h, b: (0, 0, 0))
    kv_spec = pl.BlockSpec((1, HPS, sk, dh), lambda h, b: (b, h, 0, 0))
    wq_spec = pl.BlockSpec((d_model, w), lambda h, b: (0, h))
    wo_spec = pl.BlockSpec((w, d_model), lambda h, b: (h, 0))
    out_spec = pl.BlockSpec((nb, sq, 2 * d_model), lambda h, b: (0, 0, 0))

    return pl.pallas_call(
        functools.partial(_kernel, dh=dh, d_model=d_model, scale=dh ** -0.5),
        grid=(nhp, nb),
        in_specs=[x_spec, kv_spec, kv_spec, wq_spec, wo_spec] * 2,
        out_specs=out_spec,
        out_shape=jax.ShapeDtypeStruct((nb, sq, 2 * d_model), A_x.dtype),
        scratch_shapes=[pltpu.VMEM((nb, sq, 2 * d_model), jnp.float32)],
        compiler_params=pltpu.CompilerParams(
            dimension_semantics=("arbitrary", "arbitrary"),
            vmem_limit_bytes=100 * 1024 * 1024,
        ),
    )(A_x, A_k_cache, A_v_cache, A_wq, A_wo,
      B_x, B_k_cache, B_v_cache, B_wq, B_wo)
```

```python
import functools

import jax
import jax.numpy as jnp
import jax.experimental.pallas as pl
import jax.experimental.pallas.tpu as pltpu

HPS = 2


def _kernel(ax_ref, ak_ref, av_ref, awq_ref, awo_ref,
            bx_ref, bk_ref, bv_ref, bwq_ref, bwo_ref,
            o_ref, acc_ref, *, dh, d_model, scale):
    hp = pl.program_id(0)
    b = pl.program_id(1)
    nhp = pl.num_programs(0)

    for prob, (x_ref, k_ref, v_ref, wq_ref, wo_ref) in enumerate((
            (ax_ref, ak_ref, av_ref, awq_ref, awo_ref),
            (bx_ref, bk_ref, bv_ref, bwq_ref, bwo_ref))):
        x = x_ref[b]
        q = jnp.dot(x, wq_ref[...], preferred_element_type=jnp.float32)
        q = (q * scale).astype(jnp.bfloat16)
        outs = []
        for j in range(HPS):
            qj = q[:, j * dh:(j + 1) * dh]
            s = jnp.dot(qj, k_ref[0, j], preferred_element_type=jnp.float32)
            m = jnp.max(s, axis=-1, keepdims=True)
            p = jnp.exp(s - m)
            l = jnp.sum(p, axis=-1, keepdims=True)
            oj = jax.lax.dot_general(p.astype(jnp.bfloat16), v_ref[0, j],
                                     (((1,), (1,)), ((), ())),
                                     preferred_element_type=jnp.float32)
            outs.append((oj / l).astype(jnp.bfloat16))
        o = jnp.concatenate(outs, axis=-1)
        contrib = jnp.dot(o, wo_ref[...], preferred_element_type=jnp.float32)
        cols = slice(prob * d_model, (prob + 1) * d_model)

        @pl.when(hp == 0)
        def _():
            acc_ref[b, :, cols] = contrib

        @pl.when(hp > 0)
        def _():
            acc_ref[b, :, cols] += contrib

    @pl.when(hp == nhp - 1)
    def _():
        o_ref[b] = acc_ref[b].astype(o_ref.dtype)


@jax.jit
def pallas_concat_heads__gqa_block_cached__gqa_block_cached__near_ridge_kernel(
    A_x: jax.Array,
    A_k_cache: jax.Array,
    A_v_cache: jax.Array,
    A_wq: jax.Array,
    A_wo: jax.Array,
    B_x: jax.Array,
    B_k_cache: jax.Array,
    B_v_cache: jax.Array,
    B_wq: jax.Array,
    B_wo: jax.Array,
):
    nb, sq, d_model = A_x.shape
    _, hkv, sk, dh = A_k_cache.shape
    hq = A_wq.shape[1] // dh
    assert hq == hkv and hq % HPS == 0
    nhp = hq // HPS
    w = HPS * dh

    x_spec = pl.BlockSpec((nb, sq, d_model), lambda h, b: (0, 0, 0))
    kv_spec = pl.BlockSpec((1, HPS, dh, sk), lambda h, b: (b, h, 0, 0))
    wq_spec = pl.BlockSpec((d_model, w), lambda h, b: (0, h))
    wo_spec = pl.BlockSpec((w, d_model), lambda h, b: (h, 0))
    out_spec = pl.BlockSpec((nb, sq, 2 * d_model), lambda h, b: (0, 0, 0))

    return pl.pallas_call(
        functools.partial(_kernel, dh=dh, d_model=d_model, scale=dh ** -0.5),
        grid=(nhp, nb),
        in_specs=[x_spec, kv_spec, kv_spec, wq_spec, wo_spec] * 2,
        out_specs=out_spec,
        out_shape=jax.ShapeDtypeStruct((nb, sq, 2 * d_model), A_x.dtype),
        scratch_shapes=[pltpu.VMEM((nb, sq, 2 * d_model), jnp.float32)],
        compiler_params=pltpu.CompilerParams(
            dimension_semantics=("arbitrary", "arbitrary"),
            vmem_limit_bytes=100 * 1024 * 1024,
        ),
    )(A_x, jnp.swapaxes(A_k_cache, 2, 3), jnp.swapaxes(A_v_cache, 2, 3), A_wq, A_wo,
      B_x, jnp.swapaxes(B_k_cache, 2, 3), jnp.swapaxes(B_v_cache, 2, 3), B_wq, B_wo)
```

```python
import functools

import jax
import jax.numpy as jnp
import jax.experimental.pallas as pl
import jax.experimental.pallas.tpu as pltpu

HPS = 4

_NT = (((1,), (1,)), ((), ()))


def _kernel(ax_ref, ak_ref, av_ref, awq_ref, awo_ref,
            bx_ref, bk_ref, bv_ref, bwq_ref, bwo_ref,
            o_ref, acc_ref, *, dh, d_model, scale):
    hp = pl.program_id(0)
    b = pl.program_id(1)
    nhp = pl.num_programs(0)

    @pl.when(hp == 0)
    def _():
        acc_ref[b] = jnp.zeros(acc_ref.shape[1:], acc_ref.dtype)

    probs = ((ax_ref, ak_ref, av_ref, awq_ref, awo_ref),
             (bx_ref, bk_ref, bv_ref, bwq_ref, bwo_ref))
    qs = []
    for (x_ref, k_ref, v_ref, wq_ref, wo_ref) in probs:
        q = jnp.dot(x_ref[0], wq_ref[...], preferred_element_type=jnp.float32)
        qs.append((q * scale).astype(jnp.bfloat16))
    units = [(pr, j) for pr in range(2) for j in range(HPS)]
    S, P, L, OT = {}, {}, {}, {}

    def qk(u):
        pr, j = u
        S[u] = jnp.dot(qs[pr][:, j * dh:(j + 1) * dh], probs[pr][1][0, j],
                       preferred_element_type=jnp.float32)

    def sm(u):
        s = S.pop(u)
        m = jnp.max(s, axis=-1, keepdims=True)
        p = jnp.exp(s - m)
        L[u] = jnp.sum(p, axis=-1, keepdims=True)
        P[u] = p.astype(jnp.bfloat16)

    def pv(u):
        pr, j = u
        OT[u] = jax.lax.dot_general(probs[pr][2][0, j], P.pop(u), _NT,
                                    preferred_element_type=jnp.float32)

    def proj(pr):
        o = jnp.concatenate([OT.pop((pr, j)) for j in range(HPS)], axis=0).T
        lane = jax.lax.broadcasted_iota(jnp.int32, o.shape, 1)
        inv = 1.0 / L[(pr, 0)]
        for j in range(1, HPS):
            inv = jnp.where(lane >= j * dh, 1.0 / L[(pr, j)], inv)
        o = (o * inv).astype(jnp.bfloat16)
        contrib = jnp.dot(o, probs[pr][4][...], preferred_element_type=jnp.float32)
        acc_ref[b, :, pr * d_model:(pr + 1) * d_model] += contrib

    n = len(units)
    qk(units[0])
    for i in range(n):
        if i + 1 < n:
            qk(units[i + 1])
        if i == n - 1:
            proj(0)
        sm(units[i])
        pv(units[i])
    proj(1)

    @pl.when(hp == nhp - 1)
    def _():
        o_ref[0] = acc_ref[b].astype(o_ref.dtype)


@jax.jit
def pallas_concat_heads__gqa_block_cached__gqa_block_cached__near_ridge_kernel(
    A_x: jax.Array,
    A_k_cache: jax.Array,
    A_v_cache: jax.Array,
    A_wq: jax.Array,
    A_wo: jax.Array,
    B_x: jax.Array,
    B_k_cache: jax.Array,
    B_v_cache: jax.Array,
    B_wq: jax.Array,
    B_wo: jax.Array,
):
    nb, sq, d_model = A_x.shape
    _, hkv, sk, dh = A_k_cache.shape
    hq = A_wq.shape[1] // dh
    assert hq == hkv and hq % HPS == 0
    nhp = hq // HPS
    w = HPS * dh

    x_spec = pl.BlockSpec((1, sq, d_model), lambda h, b: (b, 0, 0))
    kv_spec = pl.BlockSpec((1, HPS, dh, sk), lambda h, b: (b, h, 0, 0))
    wq_spec = pl.BlockSpec((d_model, w), lambda h, b: (0, h))
    wo_spec = pl.BlockSpec((w, d_model), lambda h, b: (h, 0))
    out_spec = pl.BlockSpec((1, sq, 2 * d_model),
                            lambda h, b: (jnp.where(h == nhp - 1, b, 0), 0, 0))

    return pl.pallas_call(
        functools.partial(_kernel, dh=dh, d_model=d_model, scale=dh ** -0.5),
        grid=(nhp, nb),
        in_specs=[x_spec, kv_spec, kv_spec, wq_spec, wo_spec] * 2,
        out_specs=out_spec,
        out_shape=jax.ShapeDtypeStruct((nb, sq, 2 * d_model), A_x.dtype),
        scratch_shapes=[pltpu.VMEM((nb, sq, 2 * d_model), jnp.float32)],
        compiler_params=pltpu.CompilerParams(
            dimension_semantics=("arbitrary", "arbitrary"),
            vmem_limit_bytes=100 * 1024 * 1024,
        ),
    )(A_x, jnp.swapaxes(A_k_cache, 2, 3), jnp.swapaxes(A_v_cache, 2, 3), A_wq, A_wo,
      B_x, jnp.swapaxes(B_k_cache, 2, 3), jnp.swapaxes(B_v_cache, 2, 3), B_wq, B_wo)
```
